```python
import jax
import jax.numpy as jnp

def _softmax(x, axis=-1):
    return jax.nn.softmax(x, axis=axis)

def _gelu(x):
    return jax.nn.gelu(x, approximate=True)

def _silu(x):
    return jax.nn.silu(x)

def _sigmoid(x):
    return jax.nn.sigmoid(x)

def _layernorm(x, axis=-1, eps=1e-05):
    m = jnp.mean(x, axis=axis, keepdims=True)
    v = jnp.var(x, axis=axis, keepdims=True)
    return (x - m) / jnp.sqrt(v + eps)

def _scatter_add(tgt, idx, src, axis=0):
    return tgt.at[idx].add(src)

def _segment_sum(src, seg, n):
    return jax.ops.segment_sum(src, seg, n)

class _Rng:

    def __init__(self, key):
        self._k = key

    def _next(self):
        self._k, sub = jax.random.split(self._k)
        return sub

    def normal(self, shape):
        return jax.random.normal(self._next(), shape, dtype=jnp.bfloat16)

    def randint(self, lo, hi, shape):
        return jax.random.randint(self._next(), shape, lo, hi, dtype=jnp.int32)

    def uniform(self, shape, lo=0.0, hi=1.0):
        return jax.random.uniform(self._next(), shape, jnp.bfloat16, lo, hi)

    def permutation(self, n):
        return jax.random.permutation(self._next(), n)
kernel_name = 'adaLN_cond__sliding_block_cached__dense_activation_mish__decode'

def setup_inputs():
    _rng = _Rng(jax.random.key(int.from_bytes(__import__("os").urandom(4), "little")))
    _w = lambda a: (lambda t: t.astype(jnp.bfloat16) if jnp.issubdtype(t.dtype, jnp.floating) else t)(jnp.asarray(a))

    def _A_setup():
        B, Sq, D = (1, 1, 640)
        Hq, Hkv, Sk, Dh = (32, 32, 32768, 192)
        assert Hq % Hkv == 0, (Hq, Hkv)
        return {'x': _w((lambda *s: _rng.normal(s) * 0.05)(B, Sq, D)), 'k_cache': _w((lambda *s: _rng.normal(s) * 0.05)(B, Hkv, Sk, Dh)), 'v_cache': _w((lambda *s: _rng.normal(s) * 0.05)(B, Hkv, Sk, Dh)), 'wq': _w((lambda *s: _rng.normal(s) * 0.05)(D, Hq * Dh) * D ** (-0.5)), 'wo': _w((lambda *s: _rng.normal(s) * 0.05)(Hq * Dh, D) * (Hq * Dh) ** (-0.5))}
    _A_in = _A_setup()

    def _B_setup():
        B, S, D, F = (1, 1, 640, 1536)
        return {'x': _w((lambda *s: _rng.normal(s) * 0.05)(B, S, D)), 'w1': _w((lambda *s: _rng.normal(s) * 0.05)(D, F) * D ** (-0.5)), 'b1': _w((lambda *s: _rng.normal(s) * 0.05)(F)), 'w2': _w((lambda *s: _rng.normal(s) * 0.05)(F, D) * F ** (-0.5))}
    _B_in = _B_setup()
    return {'A_x': _A_in['x'], 'A_k_cache': _A_in['k_cache'], 'A_v_cache': _A_in['v_cache'], 'A_wq': _A_in['wq'], 'A_wo': _A_in['wo'], 'B_x': _B_in['x'], 'B_w1': _B_in['w1'], 'B_b1': _B_in['b1'], 'B_w2': _B_in['w2'], 'c': _w((lambda *s: _rng.normal(s) * 0.05)(1, 640)), 'w_mod': _w((lambda *s: _rng.normal(s) * 0.05)(640, 6 * 640) * 640 ** (-0.5))}

def reference(A_x, A_k_cache, A_v_cache, A_wq, A_wo, B_x, B_w1, B_b1, B_w2, c, w_mod):

    def _A_ref(x, k_cache, v_cache, wq, wo):
        B, Sq, D = x.shape
        Hq, Dh = (32, 192)
        Hkv, Sk = (k_cache.shape[1], k_cache.shape[2])
        W = min(4096, max(256, Sk // 4))
        rep = Hq // Hkv
        q = (lambda x, *d: x.transpose(*d))((x @ wq).reshape(B, Sq, Hq, Dh), 0, 2, 1, 3)
        k = jnp.repeat(k_cache[:, :, Sk - W:, :], rep, axis=1)
        v = jnp.repeat(v_cache[:, :, Sk - W:, :], rep, axis=1)
        scores = jnp.einsum('bhqd,bhkd->bhqk', q, k) * Dh ** (-0.5)
        p = _softmax(scores, axis=-1)
        o = jnp.einsum('bhqk,bhkd->bhqd', p, v)
        return (lambda x, *d: x.transpose(*d))(o, 0, 2, 1, 3).reshape(B, Sq, Hq * Dh) @ wo

    def _B_ref(x, w1, b1, w2):
        h = jnp.einsum('bsd,df->bsf', x, w1) + b1
        sp = jnp.log1p(jnp.exp(-jnp.abs(h))) + jnp.where(h > 0, h, jnp.zeros_like(h))
        act = h * jnp.tanh(sp)
        return jnp.einsum('bsf,fd->bsd', act, w2)
    x = A_x
    mod = (_silu(c) @ w_mod).reshape(c.shape[0], 6, 1, -1)
    sa, ca, ga, sb, cb, gb = (mod[:, 0].copy(), mod[:, 1].copy(), mod[:, 2].copy(), mod[:, 3].copy(), mod[:, 4].copy(), mod[:, 5].copy())
    h = _layernorm(x, axis=-1) * (1 + ca) + sa
    x = x + ga * _A_ref(h, A_k_cache, A_v_cache, A_wq, A_wo)
    h = _layernorm(x, axis=-1) * (1 + cb) + sb
    x = x + gb * _B_ref(h, B_w1, B_b1, B_w2)
    return x
```

```python
import functools

import jax
import jax.numpy as jnp
from jax import lax
import jax.experimental.pallas as pl
import jax.experimental.pallas.tpu as pltpu

D = 640
H = 32
DH = 192
F = 1536
PAIR = 2 * DH
NPAIR = H // 2
LANE = 128
SUB = 8
F32 = jnp.float32
BF16 = jnp.bfloat16

CYCLES = 24
SLABS = PAIR // 16
W2_ROWS = (384, 256, 64, 64)
W2_JUMP = (5, 3, 1, 1)
W2_VPU = 2


def _layernorm(x, eps=1e-5):
    m = jnp.mean(x, axis=-1, keepdims=True)
    d = x - m
    v = jnp.mean(d * d, axis=-1, keepdims=True)
    return d / jnp.sqrt(v + eps)


def _mish(u):
    softplus = jnp.log1p(jnp.exp(-jnp.abs(u))) + jnp.where(u > 0, u, 0.0)
    return u * jnp.tanh(softplus)


def _dot(a, b):
    return jnp.dot(a, b, preferred_element_type=F32)


def _ds(start, size, align):
    return pl.ds(start if isinstance(start, int) else pl.multiple_of(start, align), size)


def _split(i, bits):
    return i >> bits, i & ((1 << bits) - 1)


def _wait_all(buf, sem):
    pltpu.make_async_copy(buf, buf, sem).wait()


def _copy_tiles(src, dst, sem, r, c, n, queue):
    nc = src.shape[1] // LANE
    while n:
        if c == 0 and n >= nc:
            m = n // nc * nc
            idx = (_ds(r * SUB, m // nc * SUB, SUB), slice(None))
        else:
            m = min(n, nc - c)
            idx = (_ds(r * SUB, SUB, SUB), pl.ds(c * LANE, m * LANE))
        pltpu.make_async_copy(src.at[idx], dst.at[idx], sem).start(priority=queue)
        r, c, n = r + (c + m) // nc, (c + m) % nc, n - m


def _kernel(x_hbm, k_hbm, v_hbm, wq_hbm, wo_hbm, w1_hbm, b1_hbm, w2_hbm, c_hbm, wmod_hbm, o_ref,
            x_v, c_v, b1_v, wmod_v, wq_v, wo_v, w1_v, w2_v, k_v, v_v, h_s, q_s, s_s, l_s, o_s, att_s, mod_s,
            sem_w, sem_k, sem_v, sem_fence):
    sk = k_hbm.shape[2]
    window = k_v.shape[2]
    quart = window // 4
    s_c, s_x, s_b1, s_mod_a, s_wq, s_mod_b, s_wo_a, s_wo_b, s_w1, s_w2 = range(10)
    nd = D // LANE

    def fence():
        pl.semaphore_signal(sem_fence, 1)
        pl.semaphore_wait(sem_fence, 1)

    def weight(src, dst, sem, rows, first, n, pieces):
        nc = src.shape[1] // LANE
        per_step = CYCLES // 2 // len(pieces)

        def piece(s, u):
            b, k = divmod(u // 2, len(pieces))
            t, m = pieces[k]
            block = first + u % 2 * (n // 2) + s * per_step + b
            _copy_tiles(src, dst, sem_w.at[sem], block * rows + t // nc, t % nc, m, 0)
        return piece

    def cache(s, u, values):
        src, dst = (v_hbm, v_v) if values else (k_hbm, k_v)
        head, odd = _split(s, 1)
        c = (u // 6) ^ (3 * odd)
        if not values:
            sem = sem_k.at[head >> 3]
        elif isinstance(s, int) and s == 2 * H - 1:
            sem = sem_v.at[NPAIR + c]
        else:
            sem = sem_v.at[head >> 1]
        slabs, rows = pl.ds(SLABS // 2 * head + 2 * (u % 6), 2), _ds(odd * SUB, SUB, SUB)
        pltpu.make_async_copy(src.at[slabs, rows, _ds(sk - window + c * quart, quart, LANE)],
                              dst.at[slabs, rows, _ds(c * quart, quart, LANE)], sem).start(priority=1)

    def steps(lo, hi, piece, first, work=None):
        values = lo >= 2 * H

        def body(i, carry):
            for u in range(CYCLES):
                piece(lo - first + i, u)
                cache(lo - 2 * H * values + i, u, values)
            if work is not None:
                fence()
                work(i)
            return carry

        if hi - lo == 1:
            body(0, 0)
            fence()
        else:
            lax.fori_loop(0, hi - lo, body, 0)

    mod_a = weight(wmod_hbm, wmod_v, s_mod_a, 2, 0, D // 16,
                   ((0, 4), (4, 4), (8, 4), (28, 4), (32, 4), (36, 4)))
    mod_b = weight(wmod_hbm, wmod_v, s_mod_b, 2, 0, D // 16,
                   ((12, 4), (16, 2), (18, 2), (20, 4), (24, 4), (40, 2),
                    (42, 2), (44, 4), (48, 4), (52, 2), (54, 2), (56, 4)))
    mod_a_cols = 12 * LANE
    query = weight(wq_hbm, wq_v, s_wq, 1, 0, D // SUB, tuple((4 * k, 4) for k in range(12)))
    wo_pieces = ((0, 4), (4, 4), (8, 2), (10, 2), (12, 4), (16, 4))
    wo_a = weight(wo_hbm, wo_v, s_wo_a, 4, 0, 144, wo_pieces)
    wo_b = weight(wo_hbm, wo_v, s_wo_b, 4, 144, 48, wo_pieces)
    w1_a = weight(w1_hbm, w1_v, s_w1, 1, 0, D // SUB, ((0, 4), (4, 2), (6, 2)))
    w1_a_cols = 8 * LANE
    small = [functools.partial(pltpu.make_async_copy, s, d, sem_w.at[i])
             for i, s, d in ((s_c, c_hbm, c_v), (s_x, x_hbm, x_v), (s_b1, b1_hbm, b1_v))]

    row = lax.broadcasted_iota(jnp.int32, (8, PAIR), 0)
    col = lax.broadcasted_iota(jnp.int32, (8, PAIR), 1)
    own = jnp.logical_or(jnp.logical_and(row == 0, col < DH), jnp.logical_and(row == 1, col >= DH))

    def modulation(i):
        cf = c_v[...].astype(F32)
        silu_c = jnp.broadcast_to(cf * jax.nn.sigmoid(cf), (8, D)).astype(BF16)
        return _dot(silu_c, wmod_v[:, _ds(i * D, D, LANE)])

    def x0():
        return jnp.broadcast_to(x_v[...].astype(F32), (8, D))

    def first_norm(i):
        for cp in small:
            cp().wait()
        _wait_all(wmod_v.at[:, pl.ds(0, mod_a_cols)], sem_w.at[s_mod_a])
        h_s[...] = _layernorm(x0()) * (1.0 + modulation(1)) + modulation(0)

    def queries(i):
        h = h_s[...].astype(BF16)
        for p in (2 * i, 2 * i + 1):
            q_s[p] = jnp.where(own, _dot(h, wq_v[:, _ds(p * PAIR, PAIR, LANE)]), 0.0)

    def pair_of(buf, p, cols):
        return buf[pl.ds(p * SLABS, SLABS), :, cols].reshape(PAIR, cols.size)

    def scores(p, c):
        q = q_s[p].astype(BF16)
        for o in range(0, quart, quart // 2):
            cols = _ds(c * quart + o, quart // 2, LANE)
            s_s[p, :, cols] = _dot(q, pair_of(k_v, p, cols)) * DH ** -0.5

    def softmax(p):
        s = s_s[p]
        e = jnp.exp(s - jnp.max(s, axis=-1, keepdims=True))
        l_s[p] = jnp.broadcast_to(jnp.sum(e, axis=-1, keepdims=True), (8, LANE))
        s_s[p] = e
        o_s[p] = jnp.zeros((8, PAIR), F32)

    def values(p, c):
        acc = jnp.zeros((8, PAIR), F32)
        for o in range(0, quart, quart // 2):
            cols = _ds(c * quart + o, quart // 2, LANE)
            acc += lax.dot_general(s_s[p, :, cols].astype(BF16), pair_of(v_v, p, cols),
                                   (((1,), (1,)), ((), ())), preferred_element_type=F32)
        o_s[p] += acc

    def project(p):
        denom = jnp.concatenate([l_s[p]] * (PAIR // LANE), axis=1)
        o = jnp.where(own, o_s[p] / denom, 0.0).astype(BF16)
        return _dot(o, wo_v[_ds(p * PAIR, PAIR, PAIR), :])

    def wait_values(p):
        _wait_all(v_v.at[pl.ds(0, SLABS)], sem_v.at[p])

    def first_scores(first, i):
        p, j = _split(first + i, 1)
        scores(p, 2 * j)
        scores(p, 2 * j + 1)
        pl.when(j == 1)(lambda: softmax(p))

    def attend(first, i):
        p, c = _split(first + i, 2)
        pl.when(c == 0)(lambda: wait_values(p))
        values(p, c)
        scores(p + 4, c)
        pl.when(c == 3)(lambda: softmax(p + 4))

    def attend_and_modulate(i):
        attend(32, i)
        mod_s[i] = modulation(i + 2)

    def attend_and_project(i):
        p, c = _split(48 + i, 2)
        pl.when(c == 0)(lambda: wait_values(p))
        values(p, c)
        att_s[...] += project(i)

        @pl.when(i < 5)
        def _():
            att_s[...] += project(8 + i)

    def attend_twice(c, i):
        if c == 0:
            wait_values(14)
        values(14, c)
        values(14, c + 1)

    steps(0, 10, mod_a, 0)
    for cp in small:
        cp().start()
    steps(10, 12, query, 10)
    steps(12, 13, query, 10, first_norm)
    steps(13, 50, query, 10)
    steps(50, 52, mod_b, 50)
    _wait_all(wq_v, sem_w.at[s_wq])
    steps(52, 60, mod_b, 50, queries)
    _wait_all(k_v.at[pl.ds(0, 4 * SLABS)], sem_k.at[0])
    steps(60, 64, mod_b, 50, functools.partial(first_scores, 0))
    steps(64, 68, mod_b, 50, functools.partial(first_scores, 4))
    steps(68, 70, mod_b, 50)
    for i in range(1, 4):
        _wait_all(k_v.at[pl.ds(0, 4 * SLABS)], sem_k.at[i])
    steps(70, 102, wo_a, 70, functools.partial(attend, 0))
    _wait_all(wmod_v.at[:, pl.ds(mod_a_cols, 6 * D - mod_a_cols)], sem_w.at[s_mod_b])
    steps(102, 106, wo_a, 70, attend_and_modulate)
    steps(106, 118, wo_b, 106, functools.partial(attend, 36))
    _wait_all(wo_v.at[pl.ds(0, 12 * PAIR)], sem_w.at[s_wo_a])
    att_s[...] = jnp.zeros((8, D), F32)
    steps(118, 122, w1_a, 118, attend_and_project)
    _wait_all(wo_v.at[pl.ds(12 * PAIR, 4 * PAIR)], sem_w.at[s_wo_b])
    steps(122, 126, w1_a, 118, lambda i: attend_and_project(i + 4))
    steps(126, 127, w1_a, 118, functools.partial(attend_twice, 0))
    steps(127, 128, w1_a, 118, functools.partial(attend_twice, 2))

    def w1_b(r, n, queue):
        idx = (pl.ds(r * SUB, n * SUB), pl.ds(w1_a_cols, F - w1_a_cols))
        pltpu.make_async_copy(w1_hbm.at[idx], w1_v.at[idx], sem_w.at[s_w1]).start(priority=queue)

    w2_rows = [sum(W2_ROWS[:i]) for i in range(len(W2_ROWS) + 1)]

    def w2_half(half):
        out = []
        for i, jump in enumerate(W2_JUMP):
            lo, hi = ((half * F // 2 + r) // SUB * nd for r in w2_rows[i:i + 2])
            size = 2 if half == 0 and i == len(W2_ROWS) - 1 else 20
            n = (hi - lo) // size
            for j in range(n):
                t = lo + j * jump % n * size
                out.append(functools.partial(_copy_tiles, w2_hbm, w2_v, sem_w.at[s_w2 + 2 * i + half],
                                             t // nd, t % nd, size))
        return out

    mid = D // SUB // 2
    queues = ([functools.partial(w1_b, r + half, 1) for r in range(14) for half in (0, mid)]
              + [functools.partial(w1_b, r, 2) for r in range(14, mid, 2)] + w2_half(1),
              [functools.partial(w1_b, mid + r, 2) for r in range(14, mid, 2)] + w2_half(0))
    todo = [functools.partial(q[j], i) for j in range(max(map(len, queues)))
            for i, q in enumerate(queues) if j < len(q)]

    def start(n):
        for cp in todo[:n]:
            cp()
        del todo[:n]
        fence()

    start(32)
    att = att_s[...] + project(13) + project(14)
    fence()
    start(12)
    _wait_all(v_v.at[pl.ds(0, SLABS * 3 // 4)], sem_v.at[NPAIR - 1])
    for c in (3, 2, 1, 0):
        _wait_all(v_v.at[pl.ds(0, SLABS // 4), :, pl.ds(0, quart)], sem_v.at[NPAIR + c])
        values(15, c)
        fence()
        start(12)

    att = jnp.broadcast_to(jnp.sum(att + project(15), axis=0, keepdims=True), (8, D))
    x1 = x0() + mod_s[0] * att
    h2 = (_layernorm(x1) * (1.0 + mod_s[2]) + mod_s[1]).astype(BF16)
    start(len(todo))
    _wait_all(w1_v, sem_w.at[s_w1])
    b1 = b1_v[...].astype(F32)
    bias = jnp.concatenate([jnp.broadcast_to(b1[t:t + 1, :], (8, LANE)) for t in range(F // LANE)], axis=1)
    act = _mish(_dot(h2, w1_v[...]) + bias).astype(BF16)
    tall = [jnp.broadcast_to(act[0:1, r - LANE:r].astype(F32), (LANE, LANE)).T for r in (F // 2, F)]
    y = jnp.zeros((8, D), F32)
    z = jnp.zeros((8, D), F32)
    for i in range(len(W2_ROWS)):
        for half in (1, 0):
            ra, rb = (half * F // 2 + r for r in w2_rows[i:i + 2])
            _wait_all(w2_v.at[pl.ds(ra, rb - ra)], sem_w.at[s_w2 + 2 * i + half])
            if i < len(W2_ROWS) - W2_VPU:
                y += _dot(act[:, ra:rb], w2_v[ra:rb, :])
                continue
            for r in range(ra, rb, 16):
                a = tall[half][r % LANE:r % LANE + 16, :]
                t = jnp.concatenate([a] * nd, axis=1) * w2_v[r:r + 16, :].astype(F32)
                z += t[:8] + t[8:]
    y = y[0:1] + jnp.sum(z, axis=0, keepdims=True)
    o_ref[...] = (x1[0:1] + mod_s[3, 0:1] * y).astype(o_ref.dtype)


@jax.jit
def pallas_adaLN_cond__sliding_block_cached__dense_activation_mish__decode_kernel(
    A_x: jax.Array,
    A_k_cache: jax.Array,
    A_v_cache: jax.Array,
    A_wq: jax.Array,
    A_wo: jax.Array,
    B_x: jax.Array,
    B_w1: jax.Array,
    B_b1: jax.Array,
    B_w2: jax.Array,
    c: jax.Array,
    w_mod: jax.Array,
):
    del B_x
    sk = A_k_cache.shape[2]
    window = min(4096, max(256, sk // 4))
    kt = jnp.swapaxes(A_k_cache, 2, 3).reshape(NPAIR * SLABS, 16, sk)
    vt = jnp.swapaxes(A_v_cache, 2, 3).reshape(NPAIR * SLABS, 16, sk)
    hbm = pl.BlockSpec(memory_space=pltpu.HBM)
    out = pl.pallas_call(
        _kernel,
        out_shape=jax.ShapeDtypeStruct((1, D), A_x.dtype),
        in_specs=[hbm] * 10,
        out_specs=pl.BlockSpec(memory_space=pltpu.VMEM),
        scratch_shapes=[
            pltpu.VMEM((1, D), BF16),
            pltpu.VMEM((1, D), BF16),
            pltpu.VMEM((F // LANE, LANE), BF16),
            pltpu.VMEM((D, 6 * D), BF16),
            pltpu.VMEM((D, H * DH), BF16),
            pltpu.VMEM((H * DH, D), BF16),
            pltpu.VMEM((D, F), BF16),
            pltpu.VMEM((F, D), BF16),
            pltpu.VMEM((NPAIR * SLABS, 16, window), BF16),
            pltpu.VMEM((NPAIR * SLABS, 16, window), BF16),
            pltpu.VMEM((8, D), F32),
            pltpu.VMEM((NPAIR, 8, PAIR), F32),
            pltpu.VMEM((NPAIR, 8, window), F32),
            pltpu.VMEM((NPAIR, 8, LANE), F32),
            pltpu.VMEM((NPAIR, 8, PAIR), F32),
            pltpu.VMEM((8, D), F32),
            pltpu.VMEM((4, 8, D), F32),
            pltpu.SemaphoreType.DMA((9 + 2 * len(W2_ROWS),)),
            pltpu.SemaphoreType.DMA((4,)),
            pltpu.SemaphoreType.DMA((NPAIR + 4,)),
            pltpu.SemaphoreType.REGULAR,
        ],
        compiler_params=pltpu.CompilerParams(
            vmem_limit_bytes=126 * 2**20,
            disable_semaphore_checks=True,
        ),
        name="adaln_attn_mlp_decode",
    )(A_x.reshape(1, D), kt, vt, A_wq, A_wo, B_w1, B_b1.reshape(F // LANE, LANE), B_w2, c, w_mod)
    return out.reshape(A_x.shape)
```

```python
import functools

import jax
import jax.numpy as jnp
from jax import lax
import jax.experimental.pallas as pl
import jax.experimental.pallas.tpu as pltpu

D = 640
H = 32
DH = 192
F = 1536
PAIR = 2 * DH
NPAIR = H // 2
LANE = 128
SUB = 8
F32 = jnp.float32
BF16 = jnp.bfloat16

CYCLES = 24
SLABS = PAIR // 16
W2_MXU = (384, 128, 128)
W2_VPU = (64, 32, 32)


def _layernorm(x, eps=1e-5):
    m = jnp.mean(x, axis=-1, keepdims=True)
    d = x - m
    v = jnp.mean(d * d, axis=-1, keepdims=True)
    return d / jnp.sqrt(v + eps)


def _mish(u):
    softplus = jnp.log1p(jnp.exp(-jnp.abs(u))) + jnp.where(u > 0, u, 0.0)
    return u * jnp.tanh(softplus)


def _dot(a, b):
    return jnp.dot(a, b, preferred_element_type=F32)


def _ds(start, size, align):
    return pl.ds(start if isinstance(start, int) else pl.multiple_of(start, align), size)


def _split(i, bits):
    return i >> bits, i & ((1 << bits) - 1)


def _wait_all(buf, sem):
    pltpu.make_async_copy(buf, buf, sem).wait()


def _copy_tiles(src, dst, sem, block, t, n, queue):
    nc = src.shape[2] // LANE
    while n:
        r, c = divmod(t, nc)
        if c == 0 and n >= nc:
            m = n // nc * nc
            idx = (block, pl.ds(r * SUB, m // nc * SUB), slice(None))
        else:
            m = min(n, nc - c)
            idx = (block, pl.ds(r * SUB, SUB), pl.ds(c * LANE, m * LANE))
        pltpu.make_async_copy(src.at[idx], dst.at[idx], sem).start(priority=queue)
        t, n = t + m, n - m


def _matrix(ref, first, n, cols=slice(None)):
    w = ref[pl.ds(first, n), :, cols]
    return w.reshape(n * w.shape[1], w.shape[2])


def _kernel(x_hbm, k_hbm, v_hbm, wq_hbm, wo_hbm, w1_hbm, b1_hbm, w2_hbm, c_hbm, wmod_hbm, o_ref,
            x_v, c_v, b1_v, wmod_v, wq_v, wo_v, w1_v, w2_v, k_v, v_v, h_s, q_s, s_s, l_s, o_s, att_s, mod_s,
            sem_w, sem_k, sem_v, sem_fence):
    sk = k_hbm.shape[2]
    window = k_v.shape[2]
    quart = window // 4
    s_c, s_x, s_b1, s_mod_a, s_wq, s_mod_b, s_wo_a, s_wo_b, s_w1, s_w2 = range(10)
    nd = D // LANE

    def fence():
        pl.semaphore_signal(sem_fence, 1)
        pl.semaphore_wait(sem_fence, 1)

    def weight(src, dst, sem, first, n, runs):
        per_step = 1 + runs[-1][-1][0]
        order = [(walk,) + piece for run in runs for walk in (0, 1) for piece in run]
        assert len(order) == CYCLES

        def piece(s, u):
            walk, b, t, m = order[u]
            _copy_tiles(src, dst, sem_w.at[sem], first + walk * (n // 2) + s * per_step + b, t, m, 0)
        return piece

    def cache(s, u, values):
        src, dst = (v_hbm, v_v) if values else (k_hbm, k_v)
        head, odd = _split(s, 1)
        c = (u // 6) ^ (3 * odd)
        if not values:
            sem = sem_k.at[head >> 3]
        elif isinstance(s, int) and s == 2 * H - 1:
            sem = sem_v.at[NPAIR + c]
        else:
            sem = sem_v.at[head >> 1]
        slabs, rows = pl.ds(SLABS // 2 * head + 2 * (u % 6), 2), _ds(odd * SUB, SUB, SUB)
        pltpu.make_async_copy(src.at[slabs, rows, _ds(sk - window + c * quart, quart, LANE)],
                              dst.at[slabs, rows, _ds(c * quart, quart, LANE)], sem).start(priority=1)

    def steps(lo, hi, piece, first, work=None):
        values = lo >= 2 * H

        def body(i, carry):
            for u in range(CYCLES):
                piece(lo - first + i, u)
                cache(lo - 2 * H * values + i, u, values)
                if lo == 0 and u == 2:
                    fence()
            if work is not None:
                fence()
                work(i)
            return carry

        if hi - lo == 1:
            body(0, 0)
            fence()
        else:
            lax.fori_loop(0, hi - lo, body, 0)

    mod_a = weight(wmod_hbm, wmod_v, s_mod_a, 0, D // 16,
                   [[(b, t, 4) for t in run] for b in (0, 1) for run in ((0, 4), (8, 28), (32, 36))])
    mod_b = weight(wmod_hbm, wmod_v, s_mod_b, 0, D // 16,
                   [[(0, t, m) for t, m in run] for run in (
                       ((12, 4), (16, 2), (18, 2)), ((20, 4), (24, 4)), ((40, 2), (42, 2)),
                       ((44, 4), (48, 4)), ((52, 2), (54, 2), (56, 4)))])
    query = weight(wq_hbm, wq_v, s_wq, 0, D // SUB, [[(0, t, 4), (0, t + 4, 4)] for t in range(0, 48, 8)])
    wo_runs = [[(0, 0, 4), (0, 4, 4)], [(0, 8, 2), (0, 10, 2), (0, 12, 4)], [(0, 16, 4), (1, 0, 4)],
               [(1, 4, 4), (1, 8, 2), (1, 10, 2)], [(1, 12, 4), (1, 16, 4)]]
    wo_a = weight(wo_hbm, wo_v, s_wo_a, 0, 144, wo_runs)
    wo_b = weight(wo_hbm, wo_v, s_wo_b, 144, 48, wo_runs)
    w1_a = weight(w1_hbm, w1_v, s_w1, 0, D // SUB, [[(b, 0, 4), (b, 4, 2), (b, 6, 2)] for b in range(4)])
    w1_a_cols = 8 * LANE

    def wait_modulation(sem, even, odd):
        for rows, spans in ((pl.ds(0, SUB), even), (pl.ds(SUB, SUB), odd)):
            for lo, hi in spans:
                _wait_all(wmod_v.at[:, rows, pl.ds(lo * LANE, (hi - lo) * LANE)], sem_w.at[sem])

    small = [functools.partial(pltpu.make_async_copy, s, d, sem_w.at[i])
             for i, s, d in ((s_c, c_hbm, c_v), (s_x, x_hbm, x_v), (s_b1, b1_hbm, b1_v))]

    row = lax.broadcasted_iota(jnp.int32, (8, PAIR), 0)
    col = lax.broadcasted_iota(jnp.int32, (8, PAIR), 1)
    own = jnp.logical_or(jnp.logical_and(row == 0, col < DH), jnp.logical_and(row == 1, col >= DH))

    def modulation(i):
        cf = c_v[...].astype(F32)
        silu_c = jnp.broadcast_to(cf * jax.nn.sigmoid(cf), (8, D)).astype(BF16)
        return _dot(silu_c, _matrix(wmod_v, 0, D // 16, _ds(i * D, D, LANE)))

    def x0():
        return jnp.broadcast_to(x_v[...].astype(F32), (8, D))

    def first_norm(i):
        for cp in small:
            cp().wait()
        wait_modulation(s_mod_a, ((0, 12), (28, 30)), ((0, 10),))
        h_s[...] = _layernorm(x0()) * (1.0 + modulation(1)) + modulation(0)

    def queries(i):
        h = h_s[...].astype(BF16)
        for p in (2 * i, 2 * i + 1):
            q_s[p] = jnp.where(own, _dot(h, _matrix(wq_v, 0, D // SUB, _ds(p * PAIR, PAIR, LANE))), 0.0)

    def scores(p, c):
        q = q_s[p].astype(BF16)
        for o in range(0, quart, quart // 2):
            cols = _ds(c * quart + o, quart // 2, LANE)
            s_s[p, :, cols] = _dot(q, _matrix(k_v, p * SLABS, SLABS, cols)) * DH ** -0.5

    def softmax(p):
        s = s_s[p]
        e = jnp.exp(s - jnp.max(s, axis=-1, keepdims=True))
        l_s[p] = jnp.broadcast_to(jnp.sum(e, axis=-1, keepdims=True), (8, LANE))
        s_s[p] = e
        o_s[p] = jnp.zeros((8, PAIR), F32)

    def values(p, c):
        acc = jnp.zeros((8, PAIR), F32)
        for o in range(0, quart, quart // 2):
            cols = _ds(c * quart + o, quart // 2, LANE)
            acc += lax.dot_general(s_s[p, :, cols].astype(BF16), _matrix(v_v, p * SLABS, SLABS, cols),
                                   (((1,), (1,)), ((), ())), preferred_element_type=F32)
        o_s[p] += acc

    def project(p):
        denom = jnp.concatenate([l_s[p]] * (PAIR // LANE), axis=1)
        o = jnp.where(own, o_s[p] / denom, 0.0).astype(BF16)
        return _dot(o, _matrix(wo_v, p * (PAIR // 32), PAIR // 32))

    def wait_values(p):
        _wait_all(v_v.at[pl.ds(p * SLABS, SLABS)], sem_v.at[p])

    def first_scores(first, i):
        p, j = _split(first + i, 1)
        scores(p, 2 * j)
        scores(p, 2 * j + 1)
        pl.when(j == 1)(lambda: softmax(p))

    def attend(first, i):
        p, c = _split(first + i, 2)
        pl.when(c == 0)(lambda: wait_values(p))
        values(p, c)
        scores(p + 4, c)
        pl.when(c == 3)(lambda: softmax(p + 4))

    def attend_and_modulate(i):
        attend(32, i)
        mod_s[i] = modulation(i + 2)

    def attend_and_project(i):
        p, c = _split(48 + i, 2)
        pl.when(c == 0)(lambda: wait_values(p))
        values(p, c)
        att_s[...] += project(i)

        @pl.when(i < 5)
        def _():
            att_s[...] += project(8 + i)

    def attend_twice(c, i):
        if c == 0:
            wait_values(14)
        values(14, c)
        values(14, c + 1)

    steps(0, 1, mod_a, 0)
    steps(1, 10, mod_a, 0)
    for cp in small:
        cp().start()
    steps(10, 12, query, 10)
    steps(12, 13, query, 10, first_norm)
    steps(13, 50, query, 10)
    steps(50, 52, mod_b, 50)
    _wait_all(wq_v, sem_w.at[s_wq])
    steps(52, 60, mod_b, 50, queries)
    _wait_all(k_v.at[pl.ds(0, 4 * SLABS)], sem_k.at[0])
    steps(60, 64, mod_b, 50, functools.partial(first_scores, 0))
    steps(64, 68, mod_b, 50, functools.partial(first_scores, 4))
    steps(68, 70, mod_b, 50)
    for i in range(1, 4):
        _wait_all(k_v.at[pl.ds(4 * SLABS * i, 4 * SLABS)], sem_k.at[i])
    steps(70, 102, wo_a, 70, functools.partial(attend, 0))
    wait_modulation(s_mod_b, ((12, 28),), ((10, 30),))
    steps(102, 106, wo_a, 70, attend_and_modulate)
    steps(106, 118, wo_b, 106, functools.partial(attend, 36))
    _wait_all(wo_v.at[pl.ds(0, 144)], sem_w.at[s_wo_a])
    att_s[...] = jnp.zeros((8, D), F32)
    steps(118, 122, w1_a, 118, attend_and_project)
    _wait_all(wo_v.at[pl.ds(144, 48)], sem_w.at[s_wo_b])
    steps(122, 126, w1_a, 118, lambda i: attend_and_project(i + 4))
    steps(126, 127, w1_a, 118, functools.partial(attend_twice, 0))
    steps(127, 128, w1_a, 118, functools.partial(attend_twice, 2))

    def w1_b(r, n, queue):
        idx = (pl.ds(r, n), slice(None), pl.ds(w1_a_cols, F - w1_a_cols))
        pltpu.make_async_copy(w1_hbm.at[idx], w1_v.at[idx], sem_w.at[s_w1]).start(priority=queue)

    w2_blocks = W2_MXU + W2_VPU
    w2_first = [[half * F // 2 + sum(w2_blocks[:i]) for i in range(len(w2_blocks))] for half in (0, 1)]

    def w2_half(half):
        return [functools.partial(_copy_tiles, w2_hbm, w2_v, sem_w.at[s_w2 + 2 * i + half], b, t, size)
                for i, (r, n) in enumerate(zip(w2_first[half], w2_blocks))
                for size in [2 if half == 0 and i >= len(W2_MXU) else 20]
                for b in range(r // 32, (r + n) // 32) for t in range(0, 20, size)]

    def wait_w2(i, half):
        first, n = w2_first[half][i] // 32, w2_blocks[i] // 32
        _wait_all(w2_v.at[pl.ds(first, n)], sem_w.at[s_w2 + 2 * i + half])

    mid = D // SUB // 2
    groups = [functools.partial(w1_b, r + half, 4) for half in (0, mid) for r in range(12, mid, 4)]
    queues = ([functools.partial(w1_b, r + half, 1) for r in range(12) for half in (0, mid)]
              + groups[:8] + w2_half(1), groups[8:] + w2_half(0))
    todo = [functools.partial(q[j], i) for j in range(max(map(len, queues)))
            for i, q in enumerate(queues) if j < len(q)]

    def start(n):
        for cp in todo[:n]:
            cp()
        del todo[:n]
        fence()

    start(32)
    att = att_s[...] + project(13) + project(14)
    fence()
    start(12)
    last_head = pl.ds(SLABS // 2 * (H - 1), SLABS // 2)
    _wait_all(v_v.at[pl.ds(SLABS // 2 * (H - 2), SLABS // 2)], sem_v.at[NPAIR - 1])
    _wait_all(v_v.at[last_head, pl.ds(0, SUB)], sem_v.at[NPAIR - 1])
    for c in (3, 2, 1, 0):
        _wait_all(v_v.at[last_head, pl.ds(SUB, SUB), pl.ds(c * quart, quart)], sem_v.at[NPAIR + c])
        values(15, c)
        fence()
        start(12)

    att = jnp.broadcast_to(jnp.sum(att + project(15), axis=0, keepdims=True), (8, D))
    x1 = x0() + mod_s[0] * att
    h2 = (_layernorm(x1) * (1.0 + mod_s[2]) + mod_s[1]).astype(BF16)
    start(len(todo))
    _wait_all(w1_v, sem_w.at[s_w1])
    b1 = b1_v[...].astype(F32)
    bias = jnp.concatenate([jnp.broadcast_to(b1[t:t + 1, :], (8, LANE)) for t in range(F // LANE)], axis=1)
    act = _mish(_dot(h2, _matrix(w1_v, 0, D // SUB)) + bias).astype(BF16)
    tall = [jnp.broadcast_to(act[0:1, r - LANE:r].astype(F32), (LANE, LANE)).T for r in (F // 2, F)]
    y = jnp.zeros((8, D), F32)
    for i, n in enumerate(W2_MXU):
        for half in (1, 0):
            wait_w2(i, half)
        for half in (1, 0):
            r = w2_first[half][i]
            y += _dot(act[:, r:r + n], _matrix(w2_v, r // 32, n // 32))
    y = jnp.where(lax.broadcasted_iota(jnp.int32, (8, D), 0) == 0, y, 0.0)
    for i, n in enumerate(W2_VPU, len(W2_MXU)):
        for half in (1, 0):
            wait_w2(i, half)
            for r in range(w2_first[half][i], w2_first[half][i] + n, 16):
                a = jnp.concatenate([tall[half][r % LANE:r % LANE + 16, :]] * nd, axis=1)
                t = a * w2_v[r // 32, pl.ds(r % 32, 16), :].astype(F32)
                y += t[:8] + t[8:]
    for shift in (4, 2, 1):
        y += pltpu.roll(y, shift, 0)
    out = (x1 + mod_s[3] * y).astype(o_ref.dtype)
    for t in range(nd):
        o_ref[:, t * LANE:(t + 1) * LANE] = out[0:1, t * LANE:(t + 1) * LANE]


@jax.jit
def pallas_adaLN_cond__sliding_block_cached__dense_activation_mish__decode_kernel(
    A_x: jax.Array,
    A_k_cache: jax.Array,
    A_v_cache: jax.Array,
    A_wq: jax.Array,
    A_wo: jax.Array,
    B_x: jax.Array,
    B_w1: jax.Array,
    B_b1: jax.Array,
    B_w2: jax.Array,
    c: jax.Array,
    w_mod: jax.Array,
):
    del B_x
    sk = A_k_cache.shape[2]
    window = min(4096, max(256, sk // 4))
    kt = jnp.swapaxes(A_k_cache, 2, 3).reshape(NPAIR * SLABS, 16, sk)
    vt = jnp.swapaxes(A_v_cache, 2, 3).reshape(NPAIR * SLABS, 16, sk)
    wq, wo, w1, w2, wmod = (w.reshape(-1, rows, w.shape[1]) for w, rows in (
        (A_wq, SUB), (A_wo, 32), (B_w1, SUB), (B_w2, 32), (w_mod, 16)))
    hbm = pl.BlockSpec(memory_space=pltpu.HBM)
    out = pl.pallas_call(
        _kernel,
        out_shape=jax.ShapeDtypeStruct((1, D), A_x.dtype),
        in_specs=[hbm] * 10,
        out_specs=pl.BlockSpec(memory_space=pltpu.VMEM),
        scratch_shapes=[
            pltpu.VMEM((1, D), BF16),
            pltpu.VMEM((1, D), BF16),
            pltpu.VMEM((F // LANE, LANE), BF16),
            *(pltpu.VMEM(w.shape, BF16) for w in (wmod, wq, wo, w1, w2)),
            pltpu.VMEM((NPAIR * SLABS, 16, window), BF16),
            pltpu.VMEM((NPAIR * SLABS, 16, window), BF16),
            pltpu.VMEM((8, D), F32),
            pltpu.VMEM((NPAIR, 8, PAIR), F32),
            pltpu.VMEM((NPAIR, 8, window), F32),
            pltpu.VMEM((NPAIR, 8, LANE), F32),
            pltpu.VMEM((NPAIR, 8, PAIR), F32),
            pltpu.VMEM((8, D), F32),
            pltpu.VMEM((4, 8, D), F32),
            pltpu.SemaphoreType.DMA((9 + 2 * len(W2_MXU + W2_VPU),)),
            pltpu.SemaphoreType.DMA((4,)),
            pltpu.SemaphoreType.DMA((NPAIR + 4,)),
            pltpu.SemaphoreType.REGULAR,
        ],
        compiler_params=pltpu.CompilerParams(
            vmem_limit_bytes=126 * 2**20,
            disable_semaphore_checks=True,
        ),
        name="adaln_attn_mlp_decode",
    )(A_x.reshape(1, D), kt, vt, wq, wo, w1, B_b1.reshape(F // LANE, LANE), w2, c, wmod)
    return out.reshape(A_x.shape)
```

```python
import functools

import jax
import jax.numpy as jnp
from jax import lax
import jax.experimental.pallas as pl
import jax.experimental.pallas.tpu as pltpu

D = 640
H = 32
DH = 192
F = 1536
PAIR = 2 * DH
NPAIR = H // 2
LANE = 128
SUB = 8
F32 = jnp.float32
BF16 = jnp.bfloat16

CYCLES = 24
SLABS = PAIR // 16
MOD_CUTS = (0, 12, 28, 30, 40, 60)
W2_MXU = (384, 128, 128)
W2_VPU = (64, 32, 32)


def _layernorm(x, eps=1e-5):
    m = jnp.mean(x, axis=-1, keepdims=True)
    d = x - m
    v = jnp.mean(d * d, axis=-1, keepdims=True)
    return d / jnp.sqrt(v + eps)


def _mish(u):
    softplus = jnp.log1p(jnp.exp(-jnp.abs(u))) + jnp.where(u > 0, u, 0.0)
    return u * jnp.tanh(softplus)


def _dot(a, b):
    return jnp.dot(a, b, preferred_element_type=F32)


def _ds(start, size, align):
    return pl.ds(start if isinstance(start, int) else pl.multiple_of(start, align), size)


def _split(i, bits):
    return i >> bits, i & ((1 << bits) - 1)


def _wait_all(buf, sem):
    pltpu.make_async_copy(buf, buf, sem).wait()


def _copy_tiles(src, dst, sem, block, t, n, queue):
    nc = src.shape[2] // LANE
    while n:
        r, c = divmod(t, nc)
        if c == 0 and n >= nc:
            m = n // nc * nc
            idx = (block, pl.ds(r * SUB, m // nc * SUB), slice(None))
        else:
            m = min(n, nc - c)
            idx = (block, pl.ds(r * SUB, SUB), pl.ds(c * LANE, m * LANE))
        pltpu.make_async_copy(src.at[idx], dst.at[idx], sem(t)).start(priority=queue)
        t, n = t + m, n - m


def _matrix(ref, first, n, cols=slice(None)):
    w = ref[pl.ds(first, n), :, cols]
    return w.reshape(n * w.shape[1], w.shape[2])


def _kernel(x_hbm, k_hbm, v_hbm, wq_hbm, wo_hbm, w1_hbm, b1_hbm, w2_hbm, c_hbm, wmod_hbm, o_ref,
            x_v, c_v, b1_v, wmod_v, wq_v, wo_v, w1_v, w2_v, k_v, v_v, h_s, q_s, s_s, l_s, o_s, att_s, mod_s,
            sem_w, sem_mod, sem_k, sem_v, sem_fence):
    sk = k_hbm.shape[2]
    window = k_v.shape[2]
    quart = window // 4
    s_c, s_x, s_b1, s_wq, s_wo_a, s_wo_b, s_w1, s_w2 = range(8)
    nd = D // LANE

    def fence():
        pl.semaphore_signal(sem_fence, 1)
        pl.semaphore_wait(sem_fence, 1)

    def weight(src, dst, sem, first, n, runs):
        per_step = 1 + runs[-1][-1][0]
        order = [(walk,) + piece for run in runs for walk in (0, 1) for piece in run]
        assert len(order) == CYCLES

        def piece(s, u):
            walk, b, t, m = order[u]
            _copy_tiles(src, dst, sem, first + walk * (n // 2) + s * per_step + b, t, m, 0)
        return piece

    def cache(s, u, values):
        src, dst = (v_hbm, v_v) if values else (k_hbm, k_v)
        head, odd = _split(s, 1)
        c = (u // 6) ^ (3 * odd)
        if not values:
            sem = sem_k.at[head >> 3]
        elif isinstance(s, int) and head == H - 1:
            sem = sem_v.at[NPAIR + (c if odd else 4)]
        else:
            sem = sem_v.at[head >> 1]
        slabs, rows = pl.ds(SLABS // 2 * head + 2 * (u % 6), 2), _ds(odd * SUB, SUB, SUB)
        pltpu.make_async_copy(src.at[slabs, rows, _ds(sk - window + c * quart, quart, LANE)],
                              dst.at[slabs, rows, _ds(c * quart, quart, LANE)], sem).start(priority=1)

    def steps(lo, hi, piece, first, work=None):
        values = lo >= 2 * H

        def body(i, carry):
            for u in range(CYCLES):
                piece(lo - first + i, u)
                cache(lo - 2 * H * values + i, u, values)
                if lo == 0 and u == 2:
                    fence()
            if work is not None:
                fence()
                work(i)
            return carry

        if hi - lo == 1:
            body(0, 0)
            fence()
        else:
            lax.fori_loop(0, hi - lo, body, 0)

    def one(i):
        return lambda t: sem_w.at[i]

    def mod_part(t):
        return sem_mod.at[sum(t >= cut for cut in MOD_CUTS[1:])]

    def wait_modulation(*parts):
        for i in parts:
            r, c = divmod(MOD_CUTS[i], 6 * nd)
            cols = pl.ds(c * LANE, (MOD_CUTS[i + 1] - MOD_CUTS[i]) * LANE)
            _wait_all(wmod_v.at[:, pl.ds(r * SUB, SUB), cols], sem_mod.at[i])

    mod_a = weight(wmod_hbm, wmod_v, mod_part, 0, D // 16,
                   [[(b, t, 4) for t in run] for b in (0, 1) for run in ((0, 4), (8, 28), (32, 36))])
    mod_b = weight(wmod_hbm, wmod_v, mod_part, 0, D // 16,
                   [[(0, t, m) for t, m in run] for run in (
                       ((12, 4), (16, 2), (18, 2)), ((20, 4), (24, 4)), ((40, 2), (42, 2)),
                       ((44, 4), (48, 4)), ((52, 2), (54, 2), (56, 4)))])
    query = weight(wq_hbm, wq_v, one(s_wq), 0, D // SUB, [[(0, t, 4), (0, t + 4, 4)] for t in range(0, 48, 8)])
    wo_runs = [[(0, 0, 4), (0, 4, 4)], [(0, 8, 2), (0, 10, 2), (0, 12, 4)], [(0, 16, 4), (1, 0, 4)],
               [(1, 4, 4), (1, 8, 2), (1, 10, 2)], [(1, 12, 4), (1, 16, 4)]]
    wo_a = weight(wo_hbm, wo_v, one(s_wo_a), 0, 144, wo_runs)
    wo_b = weight(wo_hbm, wo_v, one(s_wo_b), 144, 48, wo_runs)
    w1_a = weight(w1_hbm, w1_v, one(s_w1), 0, D // SUB, [[(b, 0, 4), (b, 4, 2), (b, 6, 2)] for b in range(4)])
    w1_a_cols = 8 * LANE
    small = [functools.partial(pltpu.make_async_copy, s, d, sem_w.at[i])
             for i, s, d in ((s_c, c_hbm, c_v), (s_x, x_hbm, x_v), (s_b1, b1_hbm, b1_v))]

    row = lax.broadcasted_iota(jnp.int32, (8, PAIR), 0)
    col = lax.broadcasted_iota(jnp.int32, (8, PAIR), 1)
    own = jnp.logical_or(jnp.logical_and(row == 0, col < DH), jnp.logical_and(row == 1, col >= DH))

    def modulation(i):
        cf = c_v[...].astype(F32)
        silu_c = jnp.broadcast_to(cf * jax.nn.sigmoid(cf), (8, D)).astype(BF16)
        return _dot(silu_c, _matrix(wmod_v, 0, D // 16, _ds(i * D, D, LANE)))

    def x0():
        return jnp.broadcast_to(x_v[...].astype(F32), (8, D))

    def first_norm(i):
        for cp in small:
            cp().wait()
        wait_modulation(0, 2, 3)
        h_s[...] = _layernorm(x0()) * (1.0 + modulation(1)) + modulation(0)

    def queries(i):
        h = h_s[...].astype(BF16)
        for p in (2 * i, 2 * i + 1):
            q_s[p] = jnp.where(own, _dot(h, _matrix(wq_v, 0, D // SUB, _ds(p * PAIR, PAIR, LANE))), 0.0)

    def scores(p, c):
        q = q_s[p].astype(BF16)
        for o in range(0, quart, quart // 2):
            cols = _ds(c * quart + o, quart // 2, LANE)
            s_s[p, :, cols] = _dot(q, _matrix(k_v, p * SLABS, SLABS, cols)) * DH ** -0.5

    def softmax(p):
        s = s_s[p]
        e = jnp.exp(s - jnp.max(s, axis=-1, keepdims=True))
        l_s[p] = jnp.broadcast_to(jnp.sum(e, axis=-1, keepdims=True), (8, LANE))
        s_s[p] = e
        o_s[p] = jnp.zeros((8, PAIR), F32)

    def values(p, c):
        acc = jnp.zeros((8, PAIR), F32)
        for o in range(0, quart, quart // 2):
            cols = _ds(c * quart + o, quart // 2, LANE)
            acc += lax.dot_general(s_s[p, :, cols].astype(BF16), _matrix(v_v, p * SLABS, SLABS, cols),
                                   (((1,), (1,)), ((), ())), preferred_element_type=F32)
        o_s[p] += acc

    def project(p):
        denom = jnp.concatenate([l_s[p]] * (PAIR // LANE), axis=1)
        o = jnp.where(own, o_s[p] / denom, 0.0).astype(BF16)
        return _dot(o, _matrix(wo_v, p * (PAIR // 32), PAIR // 32))

    def wait_values(p):
        _wait_all(v_v.at[pl.ds(p * SLABS, SLABS)], sem_v.at[p])

    def first_scores(first, i):
        p, j = _split(first + i, 1)
        scores(p, 2 * j)
        scores(p, 2 * j + 1)
        pl.when(j == 1)(lambda: softmax(p))

    def attend(first, i):
        p, c = _split(first + i, 2)
        pl.when(c == 0)(lambda: wait_values(p))
        values(p, c)
        scores(p + 4, c)
        pl.when(c == 3)(lambda: softmax(p + 4))

    def attend_and_modulate(i):
        attend(32, i)
        mod_s[i] = modulation(i + 2)

    def attend_and_project(i):
        p, c = _split(48 + i, 2)
        pl.when(c == 0)(lambda: wait_values(p))
        values(p, c)
        att_s[...] += project(i)

        @pl.when(i < 5)
        def _():
            att_s[...] += project(8 + i)

    def attend_twice(c, i):
        if c == 0:
            wait_values(14)
        values(14, c)
        values(14, c + 1)

    steps(0, 1, mod_a, 0)
    steps(1, 10, mod_a, 0)
    for cp in small:
        cp().start()
    steps(10, 12, query, 10)
    steps(12, 13, query, 10, first_norm)
    steps(13, 50, query, 10)
    steps(50, 52, mod_b, 50)
    _wait_all(wq_v, sem_w.at[s_wq])
    steps(52, 60, mod_b, 50, queries)
    _wait_all(k_v.at[pl.ds(0, 4 * SLABS)], sem_k.at[0])
    steps(60, 64, mod_b, 50, functools.partial(first_scores, 0))
    steps(64, 68, mod_b, 50, functools.partial(first_scores, 4))
    steps(68, 70, mod_b, 50)
    for i in range(1, 4):
        _wait_all(k_v.at[pl.ds(4 * SLABS * i, 4 * SLABS)], sem_k.at[i])
    steps(70, 102, wo_a, 70, functools.partial(attend, 0))
    wait_modulation(1, 4)
    steps(102, 106, wo_a, 70, attend_and_modulate)
    steps(106, 118, wo_b, 106, functools.partial(attend, 36))
    _wait_all(wo_v.at[pl.ds(0, 144)], sem_w.at[s_wo_a])
    att_s[...] = jnp.zeros((8, D), F32)
    steps(118, 122, w1_a, 118, attend_and_project)
    _wait_all(wo_v.at[pl.ds(144, 48)], sem_w.at[s_wo_b])
    steps(122, 126, w1_a, 118, lambda i: attend_and_project(i + 4))
    steps(126, 127, w1_a, 118, functools.partial(attend_twice, 0))
    steps(127, 128, w1_a, 118, functools.partial(attend_twice, 2))

    def w1_b(r, n, queue):
        idx = (pl.ds(r, n), slice(None), pl.ds(w1_a_cols, F - w1_a_cols))
        pltpu.make_async_copy(w1_hbm.at[idx], w1_v.at[idx], sem_w.at[s_w1]).start(priority=queue)

    w2_blocks = W2_MXU + W2_VPU
    w2_first = [[half * F // 2 + sum(w2_blocks[:i]) for i in range(len(w2_blocks))] for half in (0, 1)]

    def w2_half(half):
        return [functools.partial(_copy_tiles, w2_hbm, w2_v, one(s_w2 + 2 * i + half), b, t, size)
                for i, (r, n) in enumerate(zip(w2_first[half], w2_blocks))
                for size in [2 if half == 0 and i >= len(W2_MXU) else 20]
                for b in range(r // 32, (r + n) // 32) for t in range(0, 20, size)]

    def wait_w2(i, half):
        first, n = w2_first[half][i] // 32, w2_blocks[i] // 32
        _wait_all(w2_v.at[pl.ds(first, n)], sem_w.at[s_w2 + 2 * i + half])

    mid = D // SUB // 2
    groups = [functools.partial(w1_b, r + half, 4) for half in (0, mid) for r in range(12, mid, 4)]
    queues = ([functools.partial(w1_b, r + half, 1) for r in range(12) for half in (0, mid)]
              + groups[:8] + w2_half(1), groups[8:] + w2_half(0))
    todo = [functools.partial(q[j], i) for j in range(max(map(len, queues)))
            for i, q in enumerate(queues) if j < len(q)]

    def start(n):
        for cp in todo[:n]:
            cp()
        del todo[:n]
        fence()

    start(32)
    att = att_s[...] + project(13) + project(14)
    fence()
    start(12)
    last_head = pl.ds(SLABS // 2 * (H - 1), SLABS // 2)
    _wait_all(v_v.at[pl.ds(SLABS // 2 * (H - 2), SLABS // 2)], sem_v.at[NPAIR - 1])
    _wait_all(v_v.at[last_head, pl.ds(0, SUB)], sem_v.at[NPAIR + 4])
    for c in (3, 2, 1, 0):
        _wait_all(v_v.at[last_head, pl.ds(SUB, SUB), pl.ds(c * quart, quart)], sem_v.at[NPAIR + c])
        values(15, c)
        fence()
        start(12)

    att = jnp.broadcast_to(jnp.sum(att + project(15), axis=0, keepdims=True), (8, D))
    x1 = x0() + mod_s[0] * att
    h2 = (_layernorm(x1) * (1.0 + mod_s[2]) + mod_s[1]).astype(BF16)
    start(len(todo))
    _wait_all(w1_v, sem_w.at[s_w1])
    b1 = b1_v[...].astype(F32)
    bias = jnp.concatenate([jnp.broadcast_to(b1[t:t + 1, :], (8, LANE)) for t in range(F // LANE)], axis=1)
    act = _mish(_dot(h2, _matrix(w1_v, 0, D // SUB)) + bias).astype(BF16)
    tall = [jnp.broadcast_to(act[0:1, r - LANE:r].astype(F32), (LANE, LANE)).T for r in (F // 2, F)]
    y = jnp.zeros((8, D), F32)
    for i, n in enumerate(W2_MXU):
        for half in (1, 0):
            wait_w2(i, half)
        for half in (1, 0):
            r = w2_first[half][i]
            y += _dot(act[:, r:r + n], _matrix(w2_v, r // 32, n // 32))
    y = jnp.where(lax.broadcasted_iota(jnp.int32, (8, D), 0) == 0, y, 0.0)
    for i, n in enumerate(W2_VPU, len(W2_MXU)):
        for half in (1, 0):
            wait_w2(i, half)
            for r in range(w2_first[half][i], w2_first[half][i] + n, 16):
                a = jnp.concatenate([tall[half][r % LANE:r % LANE + 16, :]] * nd, axis=1)
                t = a * w2_v[r // 32, pl.ds(r % 32, 16), :].astype(F32)
                y += t[:8] + t[8:]
    for shift in (4, 2, 1):
        y += pltpu.roll(y, shift, 0)
    out = (x1 + mod_s[3] * y).astype(o_ref.dtype)
    for t in range(nd):
        o_ref[:, t * LANE:(t + 1) * LANE] = out[0:1, t * LANE:(t + 1) * LANE]


@jax.jit
def pallas_adaLN_cond__sliding_block_cached__dense_activation_mish__decode_kernel(
    A_x: jax.Array,
    A_k_cache: jax.Array,
    A_v_cache: jax.Array,
    A_wq: jax.Array,
    A_wo: jax.Array,
    B_x: jax.Array,
    B_w1: jax.Array,
    B_b1: jax.Array,
    B_w2: jax.Array,
    c: jax.Array,
    w_mod: jax.Array,
):
    del B_x
    sk = A_k_cache.shape[2]
    window = min(4096, max(256, sk // 4))
    kt = jnp.swapaxes(A_k_cache, 2, 3).reshape(NPAIR * SLABS, 16, sk)
    vt = jnp.swapaxes(A_v_cache, 2, 3).reshape(NPAIR * SLABS, 16, sk)
    wq, wo, w1, w2, wmod = (w.reshape(-1, rows, w.shape[1]) for w, rows in (
        (A_wq, SUB), (A_wo, 32), (B_w1, SUB), (B_w2, 32), (w_mod, 16)))
    hbm = pl.BlockSpec(memory_space=pltpu.HBM)
    out = pl.pallas_call(
        _kernel,
        out_shape=jax.ShapeDtypeStruct((1, D), A_x.dtype),
        in_specs=[hbm] * 10,
        out_specs=pl.BlockSpec(memory_space=pltpu.VMEM),
        scratch_shapes=[
            pltpu.VMEM((1, D), BF16),
            pltpu.VMEM((1, D), BF16),
            pltpu.VMEM((F // LANE, LANE), BF16),
            *(pltpu.VMEM(w.shape, BF16) for w in (wmod, wq, wo, w1, w2)),
            pltpu.VMEM((NPAIR * SLABS, 16, window), BF16),
            pltpu.VMEM((NPAIR * SLABS, 16, window), BF16),
            pltpu.VMEM((8, D), F32),
            pltpu.VMEM((NPAIR, 8, PAIR), F32),
            pltpu.VMEM((NPAIR, 8, window), F32),
            pltpu.VMEM((NPAIR, 8, LANE), F32),
            pltpu.VMEM((NPAIR, 8, PAIR), F32),
            pltpu.VMEM((8, D), F32),
            pltpu.VMEM((4, 8, D), F32),
            pltpu.SemaphoreType.DMA((7 + 2 * len(W2_MXU + W2_VPU),)),
            pltpu.SemaphoreType.DMA((len(MOD_CUTS) - 1,)),
            pltpu.SemaphoreType.DMA((4,)),
            pltpu.SemaphoreType.DMA((NPAIR + 5,)),
            pltpu.SemaphoreType.REGULAR,
        ],
        compiler_params=pltpu.CompilerParams(
            vmem_limit_bytes=126 * 2**20,
            disable_semaphore_checks=True,
        ),
        name="adaln_attn_mlp_decode",
    )(A_x.reshape(1, D), kt, vt, wq, wo, w1, B_b1.reshape(F // LANE, LANE), w2, c, wmod)
    return out.reshape(A_x.shape)
```
